```python
import os as _os
_os.environ.setdefault("JAX_PLATFORMS", "cpu")
import jax
import jax.numpy as jnp

def _softmax(x, axis=-1):
    return jax.nn.softmax(x, axis=axis)
def _gelu(x):
    return jax.nn.gelu(x, approximate=True)
def _silu(x):
    return jax.nn.silu(x)
def _sigmoid(x):
    return jax.nn.sigmoid(x)
def _layernorm(x, axis=-1, eps=1e-5):
    m = jnp.mean(x, axis=axis, keepdims=True)
    v = jnp.var(x, axis=axis, keepdims=True)
    return (x - m) / jnp.sqrt(v + eps)
def _scatter_add(tgt, idx, src, axis=0):
    return tgt.at[idx].add(src)
def _segment_sum(src, seg, n):
    return jax.ops.segment_sum(src, seg, n)
class _Rng:
    def __init__(self, key):
        self._k = key
    def _next(self):
        self._k, sub = jax.random.split(self._k)
        return sub
    def normal(self, shape):
        return jax.random.normal(self._next(), shape, dtype=jnp.bfloat16)
    def randint(self, lo, hi, shape):
        return jax.random.randint(self._next(), shape, lo, hi, dtype=jnp.int32)
    def uniform(self, shape, lo=0.0, hi=1.0):
        return jax.random.uniform(self._next(), shape, jnp.bfloat16, lo, hi)
    def permutation(self, n):
        return jax.random.permutation(self._next(), n)


kernel_name = 'standalone__mha_block_cached__near_ridge'

def setup_inputs():
    _rng = _Rng(jax.random.key(int.from_bytes(__import__("os").urandom(4), "little")))
    _w = (lambda a: (lambda t: t.astype(jnp.bfloat16) if jnp.issubdtype(t.dtype, jnp.floating) else t)(jnp.asarray(a)))
    B, Sq, D = 8, 144, 448
    H, Sk, Dh = 16, 2048, 256
    return {
        "x": _w((lambda *s: _rng.normal(s) * 0.8)(B, Sq, D)),
        "k_cache": _w((lambda *s: _rng.normal(s) * 0.8)(B, H, Sk, Dh)),
        "v_cache": _w((lambda *s: _rng.normal(s) * 0.05)(B, H, Sk, Dh)),
        "wq": _w((lambda *s: _rng.normal(s) * 0.8)(D, H * Dh) * (D ** -0.5)),
        "wo": _w((lambda *s: _rng.normal(s) * 0.05)(H * Dh, D) * ((H * Dh) ** -0.5)),
    }

def reference(x, k_cache, v_cache, wq, wo):
    B, Sq, D = x.shape
    H, Dh = 16, 256
    q = (lambda x, *d: x.transpose(*d))((x @ wq).reshape(B, Sq, H, Dh), 0, 2, 1, 3)
    scores = jnp.einsum("bhqd,bhkd->bhqk", q, k_cache) * (Dh ** -0.5)
    p = _softmax(scores, axis=-1)
    o = jnp.einsum("bhqk,bhkd->bhqd", p, v_cache)
    return (lambda x, *d: x.transpose(*d))(o, 0, 2, 1, 3).reshape(B, Sq, H * Dh) @ wo
```

```python
import jax
import jax.numpy as jnp
from jax import lax
import jax.experimental.pallas as pl
import jax.experimental.pallas.tpu as pltpu

_NT = (((1,), (1,)), ((), ()))


@jax.jit
def pallas_standalone__mha_block_cached__near_ridge_kernel(x, k_cache, v_cache, wq, wo):
    B, Sq, D = x.shape
    _, H, Sk, Dh = k_cache.shape
    hps = 2

    def kernel(x_ref, k_ref, v_ref, wq_ref, wot_ref, o_ref, acc_ref):
        h = pl.program_id(1)

        @pl.when(h == 0)
        def _():
            acc_ref[...] = jnp.zeros_like(acc_ref)

        for j in range(hps):
            col = pl.multiple_of((h * hps + j) * Dh, Dh)
            q = jnp.dot(x_ref[...], wq_ref[:, pl.ds(col, Dh)], preferred_element_type=jnp.float32)
            q = (q.astype(jnp.bfloat16) * (Dh ** -0.5)).astype(jnp.bfloat16)
            s = lax.dot_general(q, k_ref[j], _NT, preferred_element_type=jnp.float32)
            m = jnp.max(s, axis=-1, keepdims=True)
            p = jnp.exp(s - m)
            l = jnp.sum(p, axis=-1, keepdims=True)
            o = jnp.dot(p.astype(jnp.bfloat16), v_ref[j], preferred_element_type=jnp.float32)
            o = (o / l).astype(jnp.bfloat16)
            acc_ref[...] += lax.dot_general(o, wot_ref[:, pl.ds(col, Dh)], _NT, preferred_element_type=jnp.float32)

        @pl.when(h == H // hps - 1)
        def _():
            o_ref[...] = acc_ref[...].astype(o_ref.dtype)

    return pl.pallas_call(
        kernel,
        grid=(B, H // hps),
        in_specs=[
            pl.BlockSpec((None, Sq, D), lambda b, h: (b, 0, 0)),
            pl.BlockSpec((None, hps, Sk, Dh), lambda b, h: (b, h, 0, 0)),
            pl.BlockSpec((None, hps, Sk, Dh), lambda b, h: (b, h, 0, 0)),
            pl.BlockSpec((D, H * Dh), lambda b, h: (0, 0)),
            pl.BlockSpec((D, H * Dh), lambda b, h: (0, 0)),
        ],
        out_specs=pl.BlockSpec((None, Sq, D), lambda b, h: (b, 0, 0)),
        out_shape=jax.ShapeDtypeStruct((B, Sq, D), jnp.bfloat16),
        scratch_shapes=[pltpu.VMEM((Sq, D), jnp.float32)],
        compiler_params=pltpu.CompilerParams(
            dimension_semantics=("arbitrary", "arbitrary"), vmem_limit_bytes=100 * 2**20),
    )(x, k_cache, v_cache, wq, wo.T)
```

```python
import functools

import jax
import jax.numpy as jnp
from jax import lax
import jax.experimental.pallas as pl
import jax.experimental.pallas.tpu as pltpu

_NT = (((1,), (1,)), ((), ()))
_F32 = jnp.float32
_BF16 = jnp.bfloat16

_G = 8
_HEAD_STRIDE = 2
_C = 256
_W = 128
_CUT = 16
_ROW_OFFSET = 48
_HEAD_ORDER = 7
_WEIGHT_CUT = 512
_WEIGHT_ORDER = 11
_LOOK_W = 21
_LOOK_QK = 64
_LOOK = 48
_LOOK_HEAD = 24
_OVERLAP = 56
_PROJ_AT = (1, 3, 5, 7)
_OUT_EARLY = 6
_NSEM = 8
_NWSEM = 32


def _select(cond, a, b):
    return (a if cond else b) if isinstance(cond, bool) else jnp.where(cond, a, b)


def _both(a, b):
    if a is True or b is False:
        return b
    if b is True or a is False:
        return a
    return jnp.logical_and(a, b)


def _negate(a):
    return (not a) if isinstance(a, bool) else jnp.logical_not(a)


def _guarded(cond, fn):
    if cond is True:
        fn()
    elif cond is not False:
        pl.when(cond)(fn)


def _split(items, n):
    return [items[(len(items) * q) // n:(len(items) * (q + 1)) // n] for q in range(n)]


def _kernel(x_hbm, k_hbm, v_hbm, wq_hbm, wot_hbm, o_hbm,
            xbuf, wqbuf, wotbuf, kv, qbuf, acc, acc_last, outbuf,
            scores, scores_last, row_max, o_acc, l_acc, o_head, l_head, o_prev,
            wsem, osem, esem, sem, *run_max, B, Sq, D, H, Sk, Dh):
    G, C, W, E = _G, _C, _W, _ROW_OFFSET
    NG = B * H // G
    NRND = Sk // C
    NWIN = Sk // W
    NU = C // W
    NPOS = NU * G * 2
    LAST_K = NG * NRND
    LAST_V = LAST_K + NRND
    assert NRND == G == 8 and H == G * _HEAD_STRIDE and Dh == C and 0 <= E < W
    assert _LOOK_QK >= _LOOK >= _LOOK_HEAD and _LOOK_W < _NWSEM
    out_cols = ((0, 256), (256, D))

    def head_base(g):
        return (g >> 1) * H + (g & 1)

    def decode(pos):
        u, r = divmod(pos, 2 * G)
        i, t = divmod(r, 2)
        return u, i, t

    class Round:
        def __init__(self, R, by_head=None, last_group=False):
            gk = R >> 3
            gv = gk - 1
            self.slot = R & (_NSEM - 1)
            self.j = R & (NRND - 1)
            self.row = [head_base(gk) * Sk, head_base(gv) * Sk]
            self.next_row = [head_base(gk + 1) * Sk, head_base(gv + 1) * Sk]
            if last_group:
                self.by_head, self.has_next = True, [False, False]
                self.plane = self.next_plane = [0, 1]
            else:
                self.by_head = gv >= NG - 2 if by_head is None else by_head
                self.has_next = [gk < NG - 1, gv < NG - 1]
                self.plane = [0, _select(gv == NG - 2, 2, 1)]
                self.next_plane = [0, _select(gv + 1 == NG - 2, 2, 1)]

        def locate(self, u, i, t):
            in_order = self.j * NU + u
            in_head = (_HEAD_ORDER * (u * G + i)) % NWIN
            by_head = self.by_head if t == 1 else False
            last_in_order = (self.j == NRND - 1) if u == NU - 1 else False
            if isinstance(by_head, bool):
                last = (in_head == NWIN - 1) if by_head else last_in_order
            elif in_head == NWIN - 1:
                last = jnp.logical_or(by_head, last_in_order)
            else:
                last = _both(_negate(by_head), last_in_order)
            return _select(by_head, self.j, i), _select(by_head, in_head, in_order), last

    def start(rd, u, i, t, cond=True):
        head, window, last = rd.locate(u, i, t)
        src = (k_hbm, v_hbm)[t]

        def copy(row, plane, r0, rows, priority, part=0):
            def go():
                pltpu.make_async_copy(
                    src.at[pl.ds(pl.multiple_of(row + head * (_HEAD_STRIDE * Sk) + r0, 8), rows)],
                    kv.at[head, plane, pl.ds(pl.multiple_of(r0, 8), rows)],
                    sem.at[rd.slot, t, part]).start(priority=priority)
            return go

        for r0, rows, priority in ((E, _CUT, 0), (E + _CUT, W - _CUT, 1)):
            whole = copy(rd.row[t], rd.plane[t], window * W + r0, rows, priority)
            if r0 + rows <= W:
                _guarded(cond, whole)
                continue
            _guarded(_both(cond, _negate(last)), whole)
            if r0 < W:
                _guarded(_both(cond, last),
                         copy(rd.row[t], rd.plane[t], Sk - W + r0, W - r0, priority))
            lo = max(r0 - W, 0)
            _guarded(_both(_both(cond, last), rd.has_next[t]),
                     copy(rd.next_row[t], rd.next_plane[t], lo, r0 + rows - W - lo, priority, 1))

    def wait_round(rd, tensors):
        def wait(t, part, heads, plane, r0, rows):
            def go():
                view = kv.at[heads, plane, pl.ds(pl.multiple_of(r0, 8), rows)]
                pltpu.make_async_copy(view, view, sem.at[rd.slot, t, part]).wait()
            return go

        for t in tensors:
            if t == 1 and rd.by_head:
                heads, r0, rows, last = rd.j, E, Sk, True
            else:
                heads, r0, rows, last = slice(None), rd.j * C + E, C, rd.j == NRND - 1
            if not E:
                last = False
            _guarded(_negate(last), wait(t, 0, heads, rd.plane[t], r0, rows))
            _guarded(last, wait(t, 0, heads, rd.plane[t], r0, rows - E))
            _guarded(_both(last, rd.has_next[t]), wait(t, 1, heads, rd.next_plane[t], 0, E))

    def load_chunk(head, plane, chunk, pins):
        nparts = max(len(pins), 1)
        bounds = [8 - (8 * q) // nparts for q in range(nparts + 1)]
        lo, hi = [], []
        for q in range(nparts):
            if pins:
                pins[q]()
            r1, r0 = bounds[q] * 16, bounds[q + 1] * 16
            for parts, r in ((lo, r0), (hi, 128 + r0)):
                parts.append(kv[head, plane, pl.ds(pl.multiple_of(chunk * C + r, 16), r1 - r0), :])
        return jnp.concatenate(lo[::-1] + hi[::-1], axis=0)

    def row_max_of(m):
        return jnp.broadcast_to(jnp.max(m, axis=1, keepdims=True), (Sq, 128))

    def qk(j, i, parity, pins, dst):
        k = load_chunk(i, 0, j, pins)
        s = lax.dot_general(qbuf[parity, i], k, _NT, preferred_element_type=_F32)
        dst[i, j] = s
        prev = jnp.where(j == 0, -jnp.inf, run_max[i][parity])
        m = jnp.maximum(prev, jnp.maximum(s[:, :128], s[:, 128:]))
        run_max[i][parity] = m
        return m

    def probs(s, m):
        p0 = jnp.exp(s[:, :128] - m)
        p1 = jnp.exp(s[:, 128:] - m)
        return p0 + p1, jnp.concatenate([p0, p1], axis=1).astype(_BF16)

    def normalize(o, l):
        r = 1.0 / jnp.broadcast_to(jnp.sum(l, axis=1, keepdims=True), (Sq, 128))
        return (o * jnp.concatenate([r, r], axis=1)).astype(_BF16)

    def pv(j, i, parity, pins):
        v = load_chunk(i, 1, j, pins)
        l, p = probs(scores[i, j], row_max_of(run_max[i][parity]))
        l_acc[parity, i] = jnp.where(j == 0, 0.0, l_acc[parity, i]) + l
        o_acc[parity, i] = (jnp.where(j == 0, 0.0, o_acc[parity, i])
                            + jnp.dot(p, v, preferred_element_type=_F32))

    def pv_head(head, plane, chunk, pins, src):
        v = load_chunk(head, plane, chunk, pins)
        if chunk == 0:
            o_prev[...] = normalize(o_head[...], l_head[...])
        l, p = probs(src[head, chunk], row_max[plane - 1, head])
        o = jnp.dot(p, v, preferred_element_type=_F32)
        if chunk == 0:
            l_head[...] = l
            o_head[...] = o
        else:
            l_head[...] += l
            o_head[...] += o

    def batch_and_col(g, i):
        flat = head_base(g) + i * _HEAD_STRIDE
        return g >> 1, pl.multiple_of((flat & (H - 1)) * Dh, Dh)

    def q_proj(g, i, parity, half):
        b, col = batch_and_col(g, i)
        xb = xbuf[pl.ds(pl.multiple_of(b * Sq, 16), Sq), :]
        w = wqbuf[:, pl.ds(pl.multiple_of(col + 128 * half, 128), 128)]
        q = jnp.dot(xb, w, preferred_element_type=_F32)
        qbuf[parity, i, :, pl.ds(128 * half, 128)] = (q * (Dh ** -0.5)).astype(_BF16)

    def out_part(g, i, half, o):
        _, col = batch_and_col(g, i)
        n0, n1 = out_cols[half]
        return lax.dot_general(o, wotbuf[n0:n1, pl.ds(col, Dh)], _NT, preferred_element_type=_F32)

    def out_proj(g, i, half, o, dst, fresh=False):
        n0, n1 = out_cols[half]
        total = _select(fresh, 0.0, dst[:, n0:n1]) + out_part(g, i, half, o)
        dst[:, n0:n1] = total
        return total

    def round_body(R, mode, look, cond):
        p = (R >> 3) - 1
        j = R & (NRND - 1)
        parity = (p + 1) & 1
        ahead = range(1, (2 * NPOS + look - 1) // NPOS + 1)
        assert len(ahead) < NRND - 1
        by_head = {"qk": False, "main": None, "head": True}[mode]
        rounds = [None] + [Round(R + d, by_head) for d in ahead]
        if mode == "head":
            v_rounds = [None] + [[Round(2 * (R + d) - LAST_K + n, last_group=True) for n in range(2)]
                                 for d in ahead]

        def starter(n):
            d, pos = divmod(n, NPOS)
            u, i, t = decode(pos)
            c = cond(d, pos, t)
            if mode != "head":
                return functools.partial(start, rounds[d], u, i, t, c)
            has_k = R + d < LAST_K
            head, piece = divmod(pos, NU * G)

            def go():
                start(rounds[d], u, i, t, _both(c, has_k))
                start(v_rounds[d][head], *divmod(piece, G), 1, _both(c, _negate(has_k)))
            return go

        now = Round(R, mode == "head")
        if mode != "head":
            now.has_next = [True, True]
        wait_round(now, (0,) if mode == "qk" else (0, 1))

        todo = [starter(NPOS + look + n) for n in range(NPOS)]
        parts = _split(todo, G if mode == "qk" else 2 * G)
        if mode != "qk":
            o_done = normalize(o_acc[parity, j], l_acc[parity, j])
        for i in range(G):
            if mode == "main":
                pv(j, i, 1 - parity, parts.pop(0))
            elif mode == "head":
                pv_head(j, 2, i, parts.pop(0), scores)
            m = qk(j, i, parity, parts.pop(0), scores_last if mode == "head" else scores)
            if mode == "head":
                row_max[0, i] = row_max_of(m)
            if i not in _PROJ_AT:
                continue
            n = _PROJ_AT.index(i)
            if n < 2 and mode != "qk":
                total = out_proj(p - 1, j, n, o_done, acc,
                                 fresh=jnp.logical_and(j == 0, (p & 1) == 1))
                n0, n1 = out_cols[n]
                outbuf[jnp.maximum(p - 1, 0) >> 1, :, n0:n1] = total.astype(outbuf.dtype)
            elif n >= 2 and mode == "head":
                out_proj(p, (j - 1) & (G - 1), n - 2, o_prev[...], acc_last, fresh=j <= 1)
            elif n >= 2:
                q_proj(p + 2, j, 1 - parity, n - 2)

    XROWS = 64
    NXB = B * Sq // XROWS
    NWB = D // 8

    def window_parts(offset, cut, size):
        parts = []
        for lo, hi, priority in ((offset, offset + cut, 0), (offset + cut, offset + size, 1)):
            if lo < size:
                parts.append((0, lo, min(hi, size) - lo, priority))
            if hi > size:
                lo = max(lo, size)
                parts.append((1, lo - size, hi - lo, priority))
        return parts

    def x_copies(n, s):
        copies = []
        for ahead, a, m, priority in window_parts(E // 16 * 8, 8, XROWS):
            rows = pl.ds((n + ahead) % NXB * XROWS + a, m)
            copies.append((pltpu.make_async_copy(x_hbm.at[rows], xbuf.at[rows], s), priority))
        return copies

    def w_copies(src, dst, n, s):
        copies = []
        for ahead, a, m, priority in window_parts(E * Dh // 8, _WEIGHT_CUT, H * Dh):
            where = (pl.ds((n * _WEIGHT_ORDER + ahead) % NWB * 8, 8), pl.ds(a, m))
            copies.append((pltpu.make_async_copy(src.at[where], dst.at[where], s), priority))
        return copies

    windows = ([functools.partial(x_copies, n) for n in range(NXB)]
               + [functools.partial(w_copies, wq_hbm, wqbuf, n) for n in range(NWB)]
               + [functools.partial(w_copies, wot_hbm, wotbuf, n) for n in range(NWB)])
    assert sorted(n * _WEIGHT_ORDER % NWB for n in range(NWB)) == list(range(NWB))

    def window(n):
        return windows[n](wsem.at[n % _NWSEM])

    def lead_copies():
        if not E:
            return []
        return [(pltpu.make_async_copy(src.at[pl.ds(i * _HEAD_STRIDE * Sk, E)],
                                       kv.at[i, t, pl.ds(0, E)], esem), i & 1)
                for i in range(G) for t, src in enumerate((k_hbm, v_hbm))]

    def start_all(copies):
        for c, priority in copies:
            c.start(priority=priority)

    def wait_all(copies):
        for c, _ in copies:
            c.wait()

    lead = lead_copies()
    first = [functools.partial(start_all, lead[n:n + 2]) for n in range(0, len(lead), 2)]
    for n in range(NPOS + _LOOK_QK):
        d, pos = divmod(n, NPOS)
        if decode(pos)[2] == 0:
            first.append(functools.partial(start, Round(d), *decode(pos)))
    first = [[]] * (len(windows) - _OVERLAP) + _split(first, _OVERLAP)

    for n in range(_LOOK_W):
        start_all(window(n))
    for n in range(len(windows)):
        wait_all(window(n))
        if n + _LOOK_W < len(windows):
            start_all(window(n + _LOOK_W))
        for go in first[n]:
            go()
        done, rest = divmod(n + 1 - NXB - NWB, NWB // G)
        if done > 0 and rest == 0:
            q_proj(0, done - 1, 0, 0)
            q_proj(0, done - 1, 0, 1)
    wait_all(lead_copies())

    def scores_round(R, carry):
        def cond(d, pos, t):
            c = (R + d) * NPOS + pos < (NRND + 1) * NPOS + _LOOK
            return c if t == 0 else jnp.logical_and(c, R + d >= NRND)
        round_body(R, "qk", _LOOK_QK, cond)
        return carry
    lax.fori_loop(0, NRND, scores_round, 0)

    def main_round(R, carry):
        round_body(R, "main", _LOOK, lambda d, pos, t: True)
        return carry
    lax.fori_loop(NRND, LAST_K - NRND, main_round, 0)

    def head_round(j, carry):
        def cond(d, pos, t):
            if d * NPOS + pos < NPOS + _LOOK:
                return (j + d) * NPOS + pos >= NPOS + _LOOK
            return True
        round_body(LAST_K - NRND + j, "head", _LOOK_HEAD, cond)
        return carry
    for i in range(G):
        row_max[1, i] = row_max_of(run_max[i][NG & 1])
    lax.fori_loop(0, NRND, head_round, 0)

    def last_round(i, todo, after_sync):
        wait_round(Round(LAST_K + i, last_group=True), (1,))
        after_sync()
        g = _select(i == 0, NG - 2, NG - 1)
        parts = _split(todo, NRND)
        for chunk in range(NRND):
            pv_head(i, 1, chunk, parts[chunk], scores_last)
            if chunk in _PROJ_AT[:2]:
                out_proj(g, (i - 1) & (G - 1), _PROJ_AT.index(chunk), o_prev[...], acc_last)

    def out_copy(b):
        return pltpu.make_async_copy(outbuf.at[b], o_hbm.at[b], osem.at[b])

    def values_round(i, carry):
        R = LAST_K + i
        todo, rounds = [], {}
        for n in range(NPOS + _LOOK_HEAD, NPOS + _LOOK_HEAD + NU * G):
            d, piece = divmod(n, NU * G)
            if d not in rounds:
                rounds[d] = Round(R + d, last_group=True)
            todo.append(functools.partial(start, rounds[d], *divmod(piece, G), 1, R + d < LAST_V))

        def early_writes():
            @pl.when(i == G - 2)
            def _():
                for b in range(_OUT_EARLY):
                    out_copy(b).start()
        last_round(i, todo, early_writes)
        return carry
    lax.fori_loop(0, G - 1, values_round, 0)

    def late_writes():
        for b in range(_OUT_EARLY, B - 1):
            out_copy(b).start()
    last_round(G - 1, [], late_writes)
    o = normalize(o_head[...], l_head[...])
    last = []
    for half, (n0, n1) in enumerate(out_cols):
        outbuf[B - 1, :, n0:n1] = (
            acc_last[:, n0:n1] + out_part(NG - 1, G - 1, half, o)).astype(outbuf.dtype)
        last.append(pltpu.make_async_copy(
            outbuf.at[B - 1, :, n0:n1], o_hbm.at[B - 1, :, n0:n1], osem.at[B - 1 + half]))
        last[-1].start()
    for b in range(B - 1):
        out_copy(b).wait()
    for c in last:
        c.wait()


@jax.jit
def pallas_standalone__mha_block_cached__near_ridge_kernel(
    x: jax.Array,
    k_cache: jax.Array,
    v_cache: jax.Array,
    wq: jax.Array,
    wo: jax.Array,
):
    B, Sq, D = x.shape
    _, H, Sk, Dh = k_cache.shape
    G, C = _G, _C
    hbm = pl.BlockSpec(memory_space=pltpu.HBM)
    return pl.pallas_call(
        functools.partial(_kernel, B=B, Sq=Sq, D=D, H=H, Sk=Sk, Dh=Dh),
        out_shape=jax.ShapeDtypeStruct((B, Sq, D), x.dtype),
        in_specs=[hbm] * 5,
        out_specs=hbm,
        scratch_shapes=[
            pltpu.VMEM((B * Sq, D), x.dtype),
            pltpu.VMEM((D, H * Dh), wq.dtype),
            pltpu.VMEM((D, H * Dh), wo.dtype),
            pltpu.VMEM((G, 3, Sk, Dh), k_cache.dtype),
            pltpu.VMEM((2, G, Sq, Dh), _BF16),
            pltpu.VMEM((Sq, D), _F32),
            pltpu.VMEM((Sq, D), _F32),
            pltpu.VMEM((B, Sq, D), x.dtype),
            pltpu.VMEM((G, Sk // C, Sq, C), _F32),
            pltpu.VMEM((G, Sk // C, Sq, C), _F32),
            pltpu.VMEM((2, G, Sq, 128), _F32),
            pltpu.VMEM((2, G, Sq, Dh), _F32),
            pltpu.VMEM((2, G, Sq, 128), _F32),
            pltpu.VMEM((Sq, Dh), _F32),
            pltpu.VMEM((Sq, 128), _F32),
            pltpu.VMEM((Sq, Dh), _BF16),
            pltpu.SemaphoreType.DMA((_NWSEM,)),
            pltpu.SemaphoreType.DMA((B + 1,)),
            pltpu.SemaphoreType.DMA(()),
            pltpu.SemaphoreType.DMA((_NSEM, 2, 2)),
        ] + [pltpu.VMEM((2, Sq, 128), _F32)] * G,
        compiler_params=pltpu.CompilerParams(
            vmem_limit_bytes=100 * 2**20,
            disable_bounds_checks=True,
            disable_semaphore_checks=True,
        ),
    )(x.reshape(B * Sq, D), k_cache.reshape(B * H * Sk, Dh), v_cache.reshape(B * H * Sk, Dh),
      wq, wo.T)
```
